```python
import jax
import jax.numpy as jnp

def _softmax(x, axis=-1):
    return jax.nn.softmax(x, axis=axis)
def _gelu(x):
    return jax.nn.gelu(x, approximate=True)
def _silu(x):
    return jax.nn.silu(x)
def _sigmoid(x):
    return jax.nn.sigmoid(x)
def _layernorm(x, axis=-1, eps=1e-5):
    m = jnp.mean(x, axis=axis, keepdims=True)
    v = jnp.var(x, axis=axis, keepdims=True)
    return (x - m) / jnp.sqrt(v + eps)
def _scatter_add(tgt, idx, src, axis=0):
    return tgt.at[idx].add(src)
def _segment_sum(src, seg, n):
    return jax.ops.segment_sum(src, seg, n)
class _Rng:
    def __init__(self, key):
        self._k = key
    def _next(self):
        self._k, sub = jax.random.split(self._k)
        return sub
    def normal(self, shape):
        return jax.random.normal(self._next(), shape, dtype=jnp.bfloat16)
    def randint(self, lo, hi, shape):
        return jax.random.randint(self._next(), shape, lo, hi, dtype=jnp.int32)
    def uniform(self, shape, lo=0.0, hi=1.0):
        return jax.random.uniform(self._next(), shape, jnp.bfloat16, lo, hi)
    def permutation(self, n):
        return jax.random.permutation(self._next(), n)


kernel_name = 'concat_heads__ssm_conv_h3__compressed_kv_cla__prompt'

def setup_inputs():
    _rng = _Rng(jax.random.key(int.from_bytes(__import__("os").urandom(4), "little")))
    _w = (lambda a: (lambda t: t.astype(jnp.bfloat16) if jnp.issubdtype(t.dtype, jnp.floating) else t)(jnp.asarray(a)))
    def _A_setup():
        B, S, D = 1, 2048, 448
        ks = 4
        return {
            "q": _w((lambda *s: _rng.normal(s) * 0.05)(B, S, D)),
            "k": _w((lambda *s: _rng.normal(s) * 0.05)(B, S, D)),
            "v": _w((lambda *s: _rng.normal(s) * 0.05)(B, S, D)),
            "shift_k": _w((lambda *s: _rng.normal(s) * 0.05)(D, ks) * 0.5),
            "ssm_k": _w((lambda *s: _rng.normal(s) * 0.05)(D, S) * (1.0 / S ** 0.5)),
            "ssm_D": _w((lambda *s: _rng.normal(s) * 0.05)(D)),
        }
    _A_in = _A_setup()

    def _B_setup():
        B, H, Sq, Sk, D, M = 1, 16, 2048, 2048, 256, 448
        Dc = 4 * D
        return {
            "x": _w((lambda *s: _rng.normal(s) * 0.05)(B, Sq, M)),
            "c_kv": _w((lambda *s: _rng.normal(s) * 0.05)(B, Sk, Dc)),
            "w_q": _w((lambda *s: _rng.normal(s) * 0.05)(M, H, D) * (M ** -0.5)),
            "w_uk": _w((lambda *s: _rng.normal(s) * 0.05)(Dc, H, D) * (Dc ** -0.5)),
            "w_uv": _w((lambda *s: _rng.normal(s) * 0.05)(Dc, H, D) * (Dc ** -0.5)),
            "w_o": _w((lambda *s: _rng.normal(s) * 0.05)(H, D, M) * ((H * D) ** -0.5)),
        }
    _B_in = _B_setup()

    return {
        "A_q": _A_in["q"],
        "A_k": _A_in["k"],
        "A_v": _A_in["v"],
        "A_shift_k": _A_in["shift_k"],
        "A_ssm_k": _A_in["ssm_k"],
        "A_ssm_D": _A_in["ssm_D"],
        "B_x": _B_in["x"],
        "B_c_kv": _B_in["c_kv"],
        "B_w_q": _B_in["w_q"],
        "B_w_uk": _B_in["w_uk"],
        "B_w_uv": _B_in["w_uv"],
        "B_w_o": _B_in["w_o"],
    }

def reference(A_q, A_k, A_v, A_shift_k, A_ssm_k, A_ssm_D, B_x, B_c_kv, B_w_q, B_w_uk, B_w_uv, B_w_o):
    def _A_ref(q, k, v, shift_k, ssm_k, ssm_D):
        B, S, D = q.shape
        ks = shift_k.shape[-1]
        k_pad = jnp.pad(k, ((0, 0), (ks - 1, 0), (0, 0)))
        k_shift = jnp.zeros_like(k)
        for t in range(ks):
            k_shift = k_shift + k_pad[:, t:t + S, :] * shift_k[:, ks - 1 - t][None, None, :]
        kv = k_shift * v
        L = 2 * S
        kv_pad = jnp.pad(kv, ((0, 0), (0, S), (0, 0)))
        kf_pad = jnp.pad(ssm_k, ((0, 0), (0, S)))
        kv_f = (lambda x, axes=(-2,-1): jnp.fft.rfft2(x.astype(jnp.float32), axes=axes))(kv_pad[:, None, :, :], axes=(1, 2))
        kf_f = (lambda x, axes=(-2,-1): jnp.fft.rfft2(x.astype(jnp.float32), axes=axes))(kf_pad[:, None, :], axes=(1, 2))
        kf_f = (lambda x, *d: x.transpose(*d))(kf_f, 1, 2, 0)
        y_f = kv_f * kf_f[None, :, :, :]
        y = (lambda x, s, axes=(-2,-1): jnp.fft.irfft2(x, s=s, axes=axes).astype(jnp.bfloat16))(y_f, (1, L), axes=(1, 2))[:, 0, :S, :]
        y = y + kv * ssm_D[None, None, :]
        return q * y

    def _B_ref(x, c_kv, w_q, w_uk, w_uv, w_o):
        B, Sq, M = x.shape[0], x.shape[1], x.shape[2]
        Sk = c_kv.shape[1]
        H, D = w_q.shape[1], w_q.shape[2]
        q = jnp.einsum("bqm,mhd->bhqd", x, w_q)
        k = jnp.einsum("bkc,chd->bhkd", c_kv, w_uk)
        v = jnp.einsum("bkc,chd->bhkd", c_kv, w_uv)
        scores = jnp.einsum("bhqd,bhkd->bhqk", q, k) * (D ** -0.5)
        off = Sk - Sq
        qi = jnp.arange(Sq)[:, None]
        kj = jnp.arange(Sk)[None, :]
        cmask = kj <= (qi + off)
        scores = jnp.where(cmask[None, None], scores, -1e9)
        p = _softmax(scores, axis=-1)
        ctx = jnp.einsum("bhqk,bhkd->bhqd", p, v)
        return jnp.einsum("bhqd,hdm->bqm", ctx, w_o)

    a = _A_ref(A_q, A_k, A_v, A_shift_k, A_ssm_k, A_ssm_D)
    b = _B_ref(B_x, B_c_kv, B_w_q, B_w_uk, B_w_uv, B_w_o)
    return jnp.concatenate([a, b], axis=-1)
```

```python
import functools
import numpy as np
import jax
import jax.numpy as jnp
from jax import lax
import jax.experimental.pallas as pl
import jax.experimental.pallas.tpu as pltpu

S = 2048
DA = 448
M = 448
H = 16
D = 256
DC = 1024
T = 128
NCH = S // T
BQ = 256
NQ = S // BQ

F32 = jnp.float32
BF16 = jnp.bfloat16


def _dft_consts():
    n = np.arange(T)
    k = np.arange(T)
    w = np.pi * (2 * k[:, None] + 1) * n[None, :] / (2 * T)
    fwd = np.concatenate([np.cos(w), -np.sin(w)], axis=0)
    inv = np.concatenate([np.cos(w).T, -np.sin(w).T], axis=1) / T
    return np.ascontiguousarray(fwd.T).astype(np.float32), np.ascontiguousarray(inv.T).astype(np.float32)


def _nt(a, b):
    return lax.dot_general(a, b, (((1,), (1,)), ((), ())), preferred_element_type=F32)


def _nn(a, b):
    return jnp.dot(a, b, preferred_element_type=F32)


def _kernel(aq_h, ak_h, av_h, shift_ref, ssmk_h, ssmd_ref, x_h, c_h, wq_h, wk_h, wv_h, wo_h,
            fwd_ref, inv_ref, out_h,
            aq, ak, av, hk, kvs, xs, gs, obuf,
            xt, x, c, wq, wk, wv, wo, wpair, wqpair, qs, ks, vs, acc, sems):
    cp = pltpu.make_async_copy
    a_copies = [cp(ssmk_h, hk, sems.at[0]), cp(ak_h, ak, sems.at[1]), cp(av_h, av, sems.at[2]),
                cp(aq_h, aq, sems.at[3])]
    b_copies = [cp(x_h, xt, sems.at[4]), cp(c_h, c, sems.at[5]), cp(wo_h, wo, sems.at[6])]
    for n_, (src, dst) in enumerate([(wq_h, wq), (wk_h, wk), (wv_h, wv)]):
        for half in range(2):
            b_copies.append(cp(src.at[:, half * 128:(half + 1) * 128], dst.at[half],
                               sems.at[12 + 2 * n_ + half]))
    for d in a_copies + b_copies:
        d.start()

    fwd = fwd_ref[...].astype(BF16)
    inv = inv_ref[...].astype(BF16)
    sgn = jnp.where((lax.broadcasted_iota(jnp.int32, (DA, T), 1) & 1) == 0, 1.0, -1.0).astype(F32)

    a_copies[0].wait()
    prev = None
    for m_ in range(NCH):
        hf = _nn(hk[:, m_ * T:(m_ + 1) * T], fwd)
        if prev is None:
            gs[m_] = hf
        else:
            gs[m_, :, :T] = hf[:, :T] - sgn * prev[:, T:]
            gs[m_, :, T:] = hf[:, T:] + sgn * prev[:, :T]
        prev = hf

    a_copies[1].wait()
    a_copies[2].wait()
    sh = shift_ref[...].astype(F32)
    shb = [jnp.broadcast_to(sh[:, s_:s_ + 1], (DA, T)) for s_ in range(4)]
    lane = lax.broadcasted_iota(jnp.int32, (DA, T), 1)
    rprev = None
    for j in range(NCH):
        kc = ak[:, j * T:(j + 1) * T].astype(F32)
        rcur = [pltpu.roll(kc, s_, 1) for s_ in range(1, 4)]
        acc_k = kc * shb[0]
        for s_ in range(1, 4):
            fill = 0.0 if rprev is None else rprev[s_ - 1]
            acc_k = acc_k + jnp.where(lane >= s_, rcur[s_ - 1], fill) * shb[s_]
        rprev = rcur
        kvb = (acc_k * av[:, j * T:(j + 1) * T].astype(F32)).astype(BF16)
        kvs[:, j * T:(j + 1) * T] = kvb
        xs[j] = _nn(kvb, fwd)

    a_copies[3].wait()
    dd = jnp.broadcast_to(ssmd_ref[...].astype(F32), (DA, T))
    R = 64
    for i in range(NCH):
        zs = []
        for r in range(0, DA, R):
            zr = jnp.zeros((R, T), F32)
            zi = jnp.zeros((R, T), F32)
            for j in range(i + 1):
                xr = xs[j, r:r + R, :T]
                xi = xs[j, r:r + R, T:]
                gr = gs[i - j, r:r + R, :T]
                gi = gs[i - j, r:r + R, T:]
                zr = zr + (xr * gr - xi * gi)
                zi = zi + (xr * gi + xi * gr)
            zs.append(jnp.concatenate([zr.astype(BF16), zi.astype(BF16)], axis=1))
        z = jnp.concatenate(zs, axis=0)
        y = _nn(z, inv)
        y = y + kvs[:, i * T:(i + 1) * T].astype(F32) * dd
        o = aq[:, i * T:(i + 1) * T].astype(F32) * y
        obuf[i * T:(i + 1) * T, 0:DA] = o.T.astype(BF16)

    out_a = cp(obuf.at[:, 0:384], out_h.at[:, 0:384], sems.at[10])
    out_a.start()

    for d in b_copies:
        d.wait()
    for r in range(0, S, 256):
        x[r:r + 256, :] = xt[:, r:r + 256].astype(F32).T.astype(BF16)
    wq32 = wq.bitcast(jnp.uint32)
    wk32 = wk.bitcast(jnp.uint32)
    wv32 = wv.bitcast(jnp.uint32)

    def unpack_pair(src32, n, j, dst, col):
        CH = 64
        for r in range(0, n, CH):
          for half in range(2):
            w = src32[half, pl.ds(r * 8 + j, CH, stride=8), :]
            lo = pltpu.bitcast(w << 16, F32)
            hi = pltpu.bitcast(w & jnp.uint32(0xFFFF0000), F32)
            c0 = col + half * 128
            dst[0, r:r + CH, c0:c0 + 128] = lo.astype(BF16)
            dst[1, r:r + CH, c0:c0 + 128] = hi.astype(BF16)

    row = lax.broadcasted_iota(jnp.int32, (BQ, BQ), 0)
    colm = lax.broadcasted_iota(jnp.int32, (BQ, BQ), 1)
    cmask = colm <= row
    acc[...] = jnp.zeros(acc.shape, F32)

    def head(h, par):
        PB = 512
        for r in range(0, S, PB):
            qs[r:r + PB, :] = (_nn(x[r:r + PB, :], wqpair[par]) * (D ** -0.5)).astype(BF16)
            kv = _nn(c[r:r + PB, :], wpair[par])
            ks[r:r + PB, :] = kv[:, :D].astype(BF16)
            vs[r:r + PB, :] = kv[:, D:].astype(BF16)
        woh = wo[h]
        for i in range(NQ):
            L = (i + 1) * BQ
            q = qs[i * BQ:(i + 1) * BQ, :]
            s_d = jnp.where(cmask, _nt(q, ks[L - BQ:L, :]), -1e9)
            mx = jnp.max(s_d, axis=1, keepdims=True)
            if i > 0:
                s_o = _nt(q, ks[0:L - BQ, :])
                mx = jnp.maximum(mx, jnp.max(s_o, axis=1, keepdims=True))
            p_d = jnp.exp(s_d - mx)
            l = jnp.sum(p_d, axis=1, keepdims=True)
            ctx = _nn(p_d.astype(BF16), vs[L - BQ:L, :])
            if i > 0:
                p_o = jnp.exp(s_o - mx)
                l = l + jnp.sum(p_o, axis=1, keepdims=True)
                ctx = ctx + _nn(p_o.astype(BF16), vs[0:L - BQ, :])
            ctx = (ctx * (1.0 / l)).astype(BF16)
            acc[i * BQ:(i + 1) * BQ, :] += _nt(ctx, woh)

    def pair(j, carry):
        for js in range(H // 2):
            @pl.when(j == js)
            def _(js=js):
                unpack_pair(wq32, M, js, wqpair, 0)
                unpack_pair(wk32, DC, js, wpair, 0)
                unpack_pair(wv32, DC, js, wpair, D)

        def hh(par, cc):
            head(2 * j + par, par)
            return cc
        lax.fori_loop(0, 2, hh, 0)
        return carry

    lax.fori_loop(0, H // 2, pair, 0)

    obuf[:, DA:] = acc[...].astype(BF16)
    out_b = cp(obuf.at[:, 384:], out_h.at[:, 384:], sems.at[11])
    out_b.start()
    out_a.wait()
    out_b.wait()


@jax.jit
def pallas_concat_heads__ssm_conv_h3__compressed_kv_cla__prompt_kernel(
    A_q, A_k, A_v, A_shift_k, A_ssm_k, A_ssm_D, B_x, B_c_kv, B_w_q, B_w_uk, B_w_uv, B_w_o,
):
    fwd, inv = _dft_consts()
    any_spec = pl.BlockSpec(memory_space=pl.ANY)
    vm = pl.BlockSpec(memory_space=pltpu.VMEM)
    out = pl.pallas_call(
        _kernel,
        out_shape=jax.ShapeDtypeStruct((S, DA + M), BF16),
        in_specs=[any_spec, any_spec, any_spec, vm, any_spec, vm,
                  any_spec, any_spec, any_spec, any_spec, any_spec, any_spec, vm, vm],
        out_specs=any_spec,
        scratch_shapes=[
            pltpu.VMEM((DA, S), BF16), pltpu.VMEM((DA, S), BF16), pltpu.VMEM((DA, S), BF16),
            pltpu.VMEM((DA, S), BF16),
            pltpu.VMEM((DA, S), BF16),
            pltpu.VMEM((NCH, DA, 2 * T), F32), pltpu.VMEM((NCH, DA, 2 * T), F32),
            pltpu.VMEM((S, DA + M), BF16),
            pltpu.VMEM((M, S), BF16), pltpu.VMEM((S, M), BF16), pltpu.VMEM((S, DC), BF16),
            pltpu.VMEM((2, M * H, 128), BF16), pltpu.VMEM((2, DC * H, 128), BF16),
            pltpu.VMEM((2, DC * H, 128), BF16),
            pltpu.VMEM((H, M, D), BF16),
            pltpu.VMEM((2, DC, 2 * D), BF16), pltpu.VMEM((2, M, D), BF16),
            pltpu.VMEM((S, D), BF16), pltpu.VMEM((S, D), BF16), pltpu.VMEM((S, D), BF16),
            pltpu.VMEM((S, M), F32),
            pltpu.SemaphoreType.DMA((18,)),
        ],
        compiler_params=pltpu.CompilerParams(vmem_limit_bytes=110 * 1024 * 1024),
    )(
        A_q.reshape(S, DA).T, A_k.reshape(S, DA).T, A_v.reshape(S, DA).T, A_shift_k, A_ssm_k,
        A_ssm_D.reshape(DA, 1), B_x.reshape(S, M).T, B_c_kv.reshape(S, DC),
        B_w_q.reshape(M * H, D), B_w_uk.reshape(DC * H, D), B_w_uv.reshape(DC * H, D), B_w_o.transpose(0, 2, 1),
        fwd, inv,
    )
    return out.reshape(1, S, DA + M)
```

```python
import functools
import numpy as np
import jax
import jax.numpy as jnp
from jax import lax
import jax.experimental.pallas as pl
import jax.experimental.pallas.tpu as pltpu

S = 2048
DA = 448
M = 448
H = 16
D = 256
DC = 1024
T = 128
NCH = S // T
BQ = 256
NQ = S // BQ

F32 = jnp.float32
BF16 = jnp.bfloat16


def _dft_consts():
    n = np.arange(T)
    k = np.arange(T)
    w = np.pi * (2 * k[:, None] + 1) * n[None, :] / (2 * T)
    fwd = np.concatenate([np.cos(w), -np.sin(w)], axis=0)
    inv = np.concatenate([np.cos(w).T, -np.sin(w).T], axis=1) / T
    return np.ascontiguousarray(fwd.T).astype(np.float32), np.ascontiguousarray(inv.T).astype(np.float32)


def _nt(a, b):
    return lax.dot_general(a, b, (((1,), (1,)), ((), ())), preferred_element_type=F32)


def _nn(a, b):
    return jnp.dot(a, b, preferred_element_type=F32)


def _kernel(aq_h, ak_h, av_h, shift_ref, ssmk_h, ssmd_ref, x_h, c_h, wq_h, wk_h, wv_h, wo_h,
            fwd_ref, inv_ref, out_h,
            aq, ak, av, hk, kvs, xs, gs, obuf,
            xt, x, c, wq, wk, wv, wo, wpair, wqpair, qs, ks, vs, acc, sems):
    cp = pltpu.make_async_copy
    a_copies = [cp(ssmk_h, hk, sems.at[0]), cp(ak_h, ak, sems.at[1]), cp(av_h, av, sems.at[2]),
                cp(aq_h, aq, sems.at[3])]
    b_copies = [cp(x_h, xt, sems.at[4]), cp(c_h, c, sems.at[5]), cp(wo_h, wo, sems.at[6])]
    for n_, (src, dst) in enumerate([(wq_h, wq), (wk_h, wk), (wv_h, wv)]):
        for half in range(2):
            b_copies.append(cp(src.at[:, half * 128:(half + 1) * 128], dst.at[half],
                               sems.at[12 + 2 * n_ + half]))
    q_copies = [b_copies[0]] + b_copies[3:5]
    b_copies = b_copies[1:3] + b_copies[5:]
    a_copies[0].start()
    for d in q_copies:
        d.start()

    fwd = fwd_ref[...].astype(BF16)
    inv = inv_ref[...].astype(BF16)
    sgn = jnp.where((lax.broadcasted_iota(jnp.int32, (DA, T), 1) & 1) == 0, 1.0, -1.0).astype(F32)

    a_copies[0].wait()
    prev = None
    for m_ in range(NCH):
        hf = _nn(hk[:, m_ * T:(m_ + 1) * T], fwd)
        if prev is None:
            gs[m_] = hf
        else:
            gs[m_, :, :T] = hf[:, :T] - sgn * prev[:, T:]
            gs[m_, :, T:] = hf[:, T:] + sgn * prev[:, :T]
        prev = hf

    for d in q_copies:
        d.wait()
    for d in a_copies[1:] + b_copies:
        d.start()
    for r in range(0, S, 256):
        x[r:r + 256, :] = xt[:, r:r + 256].astype(F32).T.astype(BF16)
    wq32 = wq.bitcast(jnp.uint32)
    wk32 = wk.bitcast(jnp.uint32)
    wv32 = wv.bitcast(jnp.uint32)

    def unpack_pair(src32, n, j, dst, col):
        CH = 64
        for r in range(0, n, CH):
          for half in range(2):
            w = src32[half, pl.ds(r * 8 + j, CH, stride=8), :]
            lo = pltpu.bitcast(w << 16, F32)
            hi = pltpu.bitcast(w & jnp.uint32(0xFFFF0000), F32)
            c0 = col + half * 128
            dst[0, r:r + CH, c0:c0 + 128] = lo.astype(BF16)
            dst[1, r:r + CH, c0:c0 + 128] = hi.astype(BF16)

    row = lax.broadcasted_iota(jnp.int32, (BQ, BQ), 0)
    colm = lax.broadcasted_iota(jnp.int32, (BQ, BQ), 1)
    cmask = colm <= row
    acc[...] = jnp.zeros(acc.shape, F32)

    def head(h, par):
        PB = 512
        for r in range(0, S, PB):
            kv = _nn(c[r:r + PB, :], wpair[par])
            ks[r:r + PB, :] = kv[:, :D].astype(BF16)
            vs[r:r + PB, :] = kv[:, D:].astype(BF16)
        woh = wo[h]
        for i in range(NQ):
            L = (i + 1) * BQ
            q = qs[h, i * BQ:(i + 1) * BQ, :]
            s_d = jnp.where(cmask, _nt(q, ks[L - BQ:L, :]), -1e9)
            mx = jnp.max(s_d, axis=1, keepdims=True)
            if i > 0:
                s_o = _nt(q, ks[0:L - BQ, :])
                mx = jnp.maximum(mx, jnp.max(s_o, axis=1, keepdims=True))
            p_d = jnp.exp(s_d - mx)
            l = jnp.sum(p_d, axis=1, keepdims=True)
            ctx = _nn(p_d.astype(BF16), vs[L - BQ:L, :])
            if i > 0:
                p_o = jnp.exp(s_o - mx)
                l = l + jnp.sum(p_o, axis=1, keepdims=True)
                ctx = ctx + _nn(p_o.astype(BF16), vs[0:L - BQ, :])
            ctx = (ctx * (1.0 / l)).astype(BF16)
            acc[i * BQ:(i + 1) * BQ, :] += _nt(ctx, woh)

    def pair(j, carry):
        for js in range(H // 2):
            @pl.when(j == js)
            def _(js=js):
                unpack_pair(wk32, DC, js, wpair, 0)
                unpack_pair(wv32, DC, js, wpair, D)

        def hh(par, cc):
            head(2 * j + par, par)
            return cc
        lax.fori_loop(0, 2, hh, 0)
        return carry

    def qpair(j, carry):
        for js in range(H // 2):
            @pl.when(j == js)
            def _(js=js):
                unpack_pair(wq32, M, js, wqpair, 0)
        for par in range(2):
            for r in range(0, S, 512):
                qs[2 * j + par, r:r + 512, :] = (
                    _nn(x[r:r + 512, :], wqpair[par]) * (D ** -0.5)).astype(BF16)
        return carry

    lax.fori_loop(0, H // 2, qpair, 0)
    a_copies[1].wait()
    a_copies[2].wait()
    sh = shift_ref[...].astype(F32)
    shb = [jnp.broadcast_to(sh[:, s_:s_ + 1], (DA, T)) for s_ in range(4)]
    lane = lax.broadcasted_iota(jnp.int32, (DA, T), 1)
    rprev = None
    for j in range(NCH):
        kc = ak[:, j * T:(j + 1) * T].astype(F32)
        rcur = [pltpu.roll(kc, s_, 1) for s_ in range(1, 4)]
        acc_k = kc * shb[0]
        for s_ in range(1, 4):
            fill = 0.0 if rprev is None else rprev[s_ - 1]
            acc_k = acc_k + jnp.where(lane >= s_, rcur[s_ - 1], fill) * shb[s_]
        rprev = rcur
        kvb = (acc_k * av[:, j * T:(j + 1) * T].astype(F32)).astype(BF16)
        kvs[:, j * T:(j + 1) * T] = kvb
        xs[j] = _nn(kvb, fwd)

    a_copies[3].wait()
    dd = jnp.broadcast_to(ssmd_ref[...].astype(F32), (DA, T))
    R = 64
    for i in range(NCH):
        zs = []
        for r in range(0, DA, R):
            zr = jnp.zeros((R, T), F32)
            zi = jnp.zeros((R, T), F32)
            for j in range(i + 1):
                xr = xs[j, r:r + R, :T]
                xi = xs[j, r:r + R, T:]
                gr = gs[i - j, r:r + R, :T]
                gi = gs[i - j, r:r + R, T:]
                zr = zr + (xr * gr - xi * gi)
                zi = zi + (xr * gi + xi * gr)
            zs.append(jnp.concatenate([zr.astype(BF16), zi.astype(BF16)], axis=1))
        z = jnp.concatenate(zs, axis=0)
        y = _nn(z, inv)
        y = y + kvs[:, i * T:(i + 1) * T].astype(F32) * dd
        o = aq[:, i * T:(i + 1) * T].astype(F32) * y
        obuf[i * T:(i + 1) * T, 0:DA] = o.T.astype(BF16)

    out_a = cp(obuf.at[:, 0:384], out_h.at[:, 0:384], sems.at[10])
    out_a.start()

    for d in b_copies:
        d.wait()
    lax.fori_loop(0, H // 2, pair, 0)

    obuf[:, DA:] = acc[...].astype(BF16)
    out_b = cp(obuf.at[:, 384:], out_h.at[:, 384:], sems.at[11])
    out_b.start()
    out_a.wait()
    out_b.wait()


@jax.jit
def pallas_concat_heads__ssm_conv_h3__compressed_kv_cla__prompt_kernel(
    A_q, A_k, A_v, A_shift_k, A_ssm_k, A_ssm_D, B_x, B_c_kv, B_w_q, B_w_uk, B_w_uv, B_w_o,
):
    fwd, inv = _dft_consts()
    any_spec = pl.BlockSpec(memory_space=pl.ANY)
    vm = pl.BlockSpec(memory_space=pltpu.VMEM)
    out = pl.pallas_call(
        _kernel,
        out_shape=jax.ShapeDtypeStruct((S, DA + M), BF16),
        in_specs=[any_spec, any_spec, any_spec, vm, any_spec, vm,
                  any_spec, any_spec, any_spec, any_spec, any_spec, any_spec, vm, vm],
        out_specs=any_spec,
        scratch_shapes=[
            pltpu.VMEM((DA, S), BF16), pltpu.VMEM((DA, S), BF16), pltpu.VMEM((DA, S), BF16),
            pltpu.VMEM((DA, S), BF16),
            pltpu.VMEM((DA, S), BF16),
            pltpu.VMEM((NCH, DA, 2 * T), F32), pltpu.VMEM((NCH, DA, 2 * T), F32),
            pltpu.VMEM((S, DA + M), BF16),
            pltpu.VMEM((M, S), BF16), pltpu.VMEM((S, M), BF16), pltpu.VMEM((S, DC), BF16),
            pltpu.VMEM((2, M * H, 128), BF16), pltpu.VMEM((2, DC * H, 128), BF16),
            pltpu.VMEM((2, DC * H, 128), BF16),
            pltpu.VMEM((H, M, D), BF16),
            pltpu.VMEM((2, DC, 2 * D), BF16), pltpu.VMEM((2, M, D), BF16),
            pltpu.VMEM((H, S, D), BF16), pltpu.VMEM((S, D), BF16), pltpu.VMEM((S, D), BF16),
            pltpu.VMEM((S, M), F32),
            pltpu.SemaphoreType.DMA((18,)),
        ],
        compiler_params=pltpu.CompilerParams(vmem_limit_bytes=110 * 1024 * 1024),
    )(
        A_q.reshape(S, DA).T, A_k.reshape(S, DA).T, A_v.reshape(S, DA).T, A_shift_k, A_ssm_k,
        A_ssm_D.reshape(DA, 1), B_x.reshape(S, M).T, B_c_kv.reshape(S, DC),
        B_w_q.reshape(M * H, D), B_w_uk.reshape(DC * H, D), B_w_uv.reshape(DC * H, D), B_w_o.transpose(0, 2, 1),
        fwd, inv,
    )
    return out.reshape(1, S, DA + M)
```

```python
import functools
import numpy as np
import jax
import jax.numpy as jnp
from jax import lax
import jax.experimental.pallas as pl
import jax.experimental.pallas.tpu as pltpu

S = 2048
DA = 448
M = 448
H = 16
D = 256
DC = 1024
T = 128
NCH = S // T
BQ = 256
NQ = S // BQ

F32 = jnp.float32
BF16 = jnp.bfloat16


def _dft_consts():
    n = np.arange(T)
    k = np.arange(T)
    w = np.pi * (2 * k[:, None] + 1) * n[None, :] / (2 * T)
    fwd = np.concatenate([np.cos(w), -np.sin(w)], axis=0)
    inv = np.concatenate([np.cos(w).T, -np.sin(w).T], axis=1) / T
    return np.ascontiguousarray(fwd.T).astype(np.float32), np.ascontiguousarray(inv.T).astype(np.float32)


def _nt(a, b):
    return lax.dot_general(a, b, (((1,), (1,)), ((), ())), preferred_element_type=F32)


def _nn(a, b):
    return jnp.dot(a, b, preferred_element_type=F32)


def _kernel(aq_h, ak_h, av_h, shift_ref, ssmk_h, ssmd_ref, x_h, c_h, wq_h, wk_h, wv_h, wo_h,
            fwd_ref, inv_ref, out_h,
            aq, ak, av, hk, kvs, xs, gs, obuf,
            xt, x, c, wq, wk, wv, wo, wpair, wqpair, qs, ks, vs, acc, sems):
    cp = pltpu.make_async_copy
    a_copies = [cp(ssmk_h, hk, sems.at[0]), cp(ak_h, ak, sems.at[1]), cp(av_h, av, sems.at[2]),
                cp(aq_h, aq, sems.at[3])]
    b_copies = [cp(x_h, xt, sems.at[4]), cp(c_h, c, sems.at[5]), cp(wo_h, wo, sems.at[6])]
    for n_, (src, dst) in enumerate([(wq_h, wq), (wk_h, wk), (wv_h, wv)]):
        for half in range(2):
            b_copies.append(cp(src.at[:, half * 128:(half + 1) * 128], dst.at[half],
                               sems.at[12 + 2 * n_ + half]))
    q_copies = [b_copies[0]] + b_copies[3:5]
    b_copies = b_copies[1:3] + b_copies[5:]
    a_copies[0].start()
    for d in q_copies:
        d.start()

    fwd = fwd_ref[...].astype(BF16)
    inv = inv_ref[...].astype(BF16)
    sgn = jnp.where((lax.broadcasted_iota(jnp.int32, (DA, T), 1) & 1) == 0, 1.0, -1.0).astype(F32)

    a_copies[0].wait()
    prev = None
    for m_ in range(NCH):
        hf = _nn(hk[:, m_ * T:(m_ + 1) * T], fwd)
        if prev is None:
            gs[m_] = hf
        else:
            gs[m_, :, :T] = hf[:, :T] - sgn * prev[:, T:]
            gs[m_, :, T:] = hf[:, T:] + sgn * prev[:, :T]
        prev = hf

    for d in q_copies:
        d.wait()
    for d in a_copies[1:] + b_copies:
        d.start()
    for r in range(0, S, 256):
        x[r:r + 256, :] = xt[:, r:r + 256].astype(F32).T.astype(BF16)
    wq32 = wq.bitcast(jnp.uint32)
    wk32 = wk.bitcast(jnp.uint32)
    wv32 = wv.bitcast(jnp.uint32)

    def unpack_pair(src32, n, j, dst, col, d0=0):
        CH = 64
        for r in range(0, n, CH):
          for half in range(2):
            w = src32[half, pl.ds(r * 8 + j, CH, stride=8), :]
            lo = pltpu.bitcast(w << 16, F32)
            hi = pltpu.bitcast(w & jnp.uint32(0xFFFF0000), F32)
            c0 = col + half * 128
            dst[d0, r:r + CH, c0:c0 + 128] = lo.astype(BF16)
            dst[d0 + 1, r:r + CH, c0:c0 + 128] = hi.astype(BF16)

    row = lax.broadcasted_iota(jnp.int32, (BQ, BQ), 0)
    colm = lax.broadcasted_iota(jnp.int32, (BQ, BQ), 1)
    cmask = colm <= row
    acc[...] = jnp.zeros(acc.shape, F32)

    def head(h, par):
        PB = 512
        for r in range(0, S, PB):
            kv = _nn(c[r:r + PB, :], wpair[h])
            ks[r:r + PB, :] = kv[:, :D].astype(BF16)
            vs[r:r + PB, :] = kv[:, D:].astype(BF16)
        woh = wo[h]
        for i in range(NQ):
            L = (i + 1) * BQ
            q = qs[h, i * BQ:(i + 1) * BQ, :]
            s_d = jnp.where(cmask, _nt(q, ks[L - BQ:L, :]), -1e9)
            mx = jnp.max(s_d, axis=1, keepdims=True)
            if i > 0:
                s_o = _nt(q, ks[0:L - BQ, :])
                mx = jnp.maximum(mx, jnp.max(s_o, axis=1, keepdims=True))
            p_d = jnp.exp(s_d - mx)
            l = jnp.sum(p_d, axis=1, keepdims=True)
            ctx = _nn(p_d.astype(BF16), vs[L - BQ:L, :])
            if i > 0:
                p_o = jnp.exp(s_o - mx)
                l = l + jnp.sum(p_o, axis=1, keepdims=True)
                ctx = ctx + _nn(p_o.astype(BF16), vs[0:L - BQ, :])
            ctx = (ctx * (1.0 / l)).astype(BF16)
            acc[i * BQ:(i + 1) * BQ, :] += _nt(ctx, woh)

    sh = shift_ref[...].astype(F32)
    shb = [jnp.broadcast_to(sh[:, s_:s_ + 1], (DA, T)) for s_ in range(4)]
    lane = lax.broadcasted_iota(jnp.int32, (DA, T), 1)
    dd = jnp.broadcast_to(ssmd_ref[...].astype(F32), (DA, T))
    R = 64
    state = {"rprev": None}

    def a_fwd(j):
        kc = ak[:, j * T:(j + 1) * T].astype(F32)
        rcur = [pltpu.roll(kc, s_, 1) for s_ in range(1, 4)]
        acc_k = kc * shb[0]
        for s_ in range(1, 4):
            fill = 0.0 if state["rprev"] is None else state["rprev"][s_ - 1]
            acc_k = acc_k + jnp.where(lane >= s_, rcur[s_ - 1], fill) * shb[s_]
        state["rprev"] = rcur
        kvb = (acc_k * av[:, j * T:(j + 1) * T].astype(F32)).astype(BF16)
        kvs[:, j * T:(j + 1) * T] = kvb
        xs[j] = _nn(kvb, fwd)

    def a_prod(i, r):
        zr = jnp.zeros((R, T), F32)
        zi = jnp.zeros((R, T), F32)
        for j in range(i + 1):
            xr = xs[j, r:r + R, :T]
            xi = xs[j, r:r + R, T:]
            gr = gs[i - j, r:r + R, :T]
            gi = gs[i - j, r:r + R, T:]
            zr = zr + (xr * gr - xi * gi)
            zi = zi + (xr * gi + xi * gr)
        return jnp.concatenate([zr.astype(BF16), zi.astype(BF16)], axis=1)

    def a_inv(i, zs):
        y = _nn(jnp.concatenate(zs, axis=0), inv)
        y = y + kvs[:, i * T:(i + 1) * T].astype(F32) * dd
        o = aq[:, i * T:(i + 1) * T].astype(F32) * y
        obuf[i * T:(i + 1) * T, 0:DA] = o.T.astype(BF16)

    unpack_pair(wq32, M, 0, wqpair, 0)
    for h in range(H):
        if h == 2:
            for d in a_copies[1:]:
                d.wait()
        if h == 8:
            for d in b_copies:
                d.wait()
        chunks = [] if h < 2 else [h - 2] if h < 14 else [2 * h - 16, 2 * h - 15]
        if h % 2 == 0 and h + 2 < H:
            unpack_pair(wq32, M, h // 2 + 1, wqpair, 0, (h + 2) % 4)
        for c_ in chunks:
            a_fwd(c_)
        zs = {c_: [] for c_ in chunks}
        for n_, r in enumerate(range(0, S, 256)):
            qs[h, r:r + 256, :] = (_nn(x[r:r + 256, :], wqpair[h % 4]) * (D ** -0.5)).astype(BF16)
            if n_ * R < DA:
                for c_ in chunks:
                    zs[c_].append(a_prod(c_, n_ * R))
            if h >= 8 and n_ == 3:
                unpack_pair(wk32, DC, h - 8, wpair, 0, 2 * (h - 8))
            if h >= 8 and n_ == 6:
                unpack_pair(wv32, DC, h - 8, wpair, D, 2 * (h - 8))
        for c_ in chunks:
            a_inv(c_, zs[c_])

    out_a = cp(obuf.at[:, 0:384], out_h.at[:, 0:384], sems.at[10])
    out_a.start()

    def hh(h, cc):
        head(h, 0)
        return cc
    lax.fori_loop(0, H, hh, 0)

    obuf[:, DA:] = acc[...].astype(BF16)
    out_b = cp(obuf.at[:, 384:], out_h.at[:, 384:], sems.at[11])
    out_b.start()
    out_a.wait()
    out_b.wait()


@jax.jit
def pallas_concat_heads__ssm_conv_h3__compressed_kv_cla__prompt_kernel(
    A_q, A_k, A_v, A_shift_k, A_ssm_k, A_ssm_D, B_x, B_c_kv, B_w_q, B_w_uk, B_w_uv, B_w_o,
):
    fwd, inv = _dft_consts()
    any_spec = pl.BlockSpec(memory_space=pl.ANY)
    vm = pl.BlockSpec(memory_space=pltpu.VMEM)
    out = pl.pallas_call(
        _kernel,
        out_shape=jax.ShapeDtypeStruct((S, DA + M), BF16),
        in_specs=[any_spec, any_spec, any_spec, vm, any_spec, vm,
                  any_spec, any_spec, any_spec, any_spec, any_spec, any_spec, vm, vm],
        out_specs=any_spec,
        scratch_shapes=[
            pltpu.VMEM((DA, S), BF16), pltpu.VMEM((DA, S), BF16), pltpu.VMEM((DA, S), BF16),
            pltpu.VMEM((DA, S), BF16),
            pltpu.VMEM((DA, S), BF16),
            pltpu.VMEM((NCH, DA, 2 * T), F32), pltpu.VMEM((NCH, DA, 2 * T), F32),
            pltpu.VMEM((S, DA + M), BF16),
            pltpu.VMEM((M, S), BF16), pltpu.VMEM((S, M), BF16), pltpu.VMEM((S, DC), BF16),
            pltpu.VMEM((2, M * H, 128), BF16), pltpu.VMEM((2, DC * H, 128), BF16),
            pltpu.VMEM((2, DC * H, 128), BF16),
            pltpu.VMEM((H, M, D), BF16),
            pltpu.VMEM((H, DC, 2 * D), BF16), pltpu.VMEM((4, M, D), BF16),
            pltpu.VMEM((H, S, D), BF16), pltpu.VMEM((S, D), BF16), pltpu.VMEM((S, D), BF16),
            pltpu.VMEM((S, M), F32),
            pltpu.SemaphoreType.DMA((18,)),
        ],
        compiler_params=pltpu.CompilerParams(vmem_limit_bytes=110 * 1024 * 1024),
    )(
        A_q.reshape(S, DA).T, A_k.reshape(S, DA).T, A_v.reshape(S, DA).T, A_shift_k, A_ssm_k,
        A_ssm_D.reshape(DA, 1), B_x.reshape(S, M).T, B_c_kv.reshape(S, DC),
        B_w_q.reshape(M * H, D), B_w_uk.reshape(DC * H, D), B_w_uv.reshape(DC * H, D), B_w_o.transpose(0, 2, 1),
        fwd, inv,
    )
    return out.reshape(1, S, DA + M)
```

```python
import functools
import numpy as np
import jax
import jax.numpy as jnp
from jax import lax
import jax.experimental.pallas as pl
import jax.experimental.pallas.tpu as pltpu

S = 2048
DA = 448
M = 448
H = 16
D = 256
DC = 1024
T = 128
NCH = S // T
BQ = 256
NQ = S // BQ

F32 = jnp.float32
BF16 = jnp.bfloat16


def _dft_consts():
    n = np.arange(T)
    k = np.arange(T)
    w = np.pi * (2 * k[:, None] + 1) * n[None, :] / (2 * T)
    fwd = np.concatenate([np.cos(w), -np.sin(w)], axis=0)
    inv = np.concatenate([np.cos(w).T, -np.sin(w).T], axis=1) / T
    return np.ascontiguousarray(fwd.T).astype(np.float32), np.ascontiguousarray(inv.T).astype(np.float32)


def _nt(a, b):
    return lax.dot_general(a, b, (((1,), (1,)), ((), ())), preferred_element_type=F32)


def _nn(a, b):
    return jnp.dot(a, b, preferred_element_type=F32)


def _kernel(aq_h, ak_h, av_h, shift_ref, ssmk_h, ssmd_ref, x_h, c_h, wq_h, wk_h, wv_h, wo_h,
            fwd_ref, inv_ref, out_h,
            aq, ak, av, hk, kvs, xs, gs, obuf,
            xt, x, c, wq, wk, wv, wo, wpair, wqpair, qs, ks, vs, acc, sems):
    cp = pltpu.make_async_copy
    a_copies = [cp(ssmk_h, hk, sems.at[0]), cp(ak_h, ak, sems.at[1]), cp(av_h, av, sems.at[2]),
                cp(aq_h, aq, sems.at[3])]
    b_copies = [cp(x_h, xt, sems.at[4]), cp(c_h, c, sems.at[5]), cp(wo_h, wo, sems.at[6])]
    for n_, (src, dst) in enumerate([(wq_h, wq), (wk_h, wk), (wv_h, wv)]):
        for half in range(2):
            b_copies.append(cp(src.at[:, half * 128:(half + 1) * 128], dst.at[half],
                               sems.at[12 + 2 * n_ + half]))
    q_copies = [b_copies[0]] + b_copies[3:5]
    b_copies = b_copies[1:3] + b_copies[5:]
    a_copies[0].start()
    for d in q_copies:
        d.start()

    fwd = fwd_ref[...].astype(BF16)
    inv = inv_ref[...].astype(BF16)
    sgn = jnp.where((lax.broadcasted_iota(jnp.int32, (DA, T), 1) & 1) == 0, 1.0, -1.0).astype(F32)

    a_copies[0].wait()
    prev = None
    for m_ in range(NCH):
        hf = _nn(hk[:, m_ * T:(m_ + 1) * T], fwd)
        if prev is None:
            gs[m_] = hf
        else:
            gs[m_, :, :T] = hf[:, :T] - sgn * prev[:, T:]
            gs[m_, :, T:] = hf[:, T:] + sgn * prev[:, :T]
        prev = hf

    for d in q_copies:
        d.wait()
    for d in a_copies[1:] + b_copies:
        d.start()
    for r in range(0, S, 256):
        x[r:r + 256, :] = xt[:, r:r + 256].astype(F32).T.astype(BF16)
    wq32 = wq.bitcast(jnp.uint32)
    wk32 = wk.bitcast(jnp.uint32)
    wv32 = wv.bitcast(jnp.uint32)

    def unpack_pair(src32, n, j, dst, col, d0=0, r0=0):
        CH = 64
        for r in range(r0, n, CH):
          for half in range(2):
            w = src32[half, pl.ds(r * 8 + j, CH, stride=8), :]
            lo = pltpu.bitcast(w << 16, F32)
            hi = pltpu.bitcast(w & jnp.uint32(0xFFFF0000), F32)
            c0 = col + half * 128
            dst[d0, r:r + CH, c0:c0 + 128] = lo.astype(BF16)
            dst[d0 + 1, r:r + CH, c0:c0 + 128] = hi.astype(BF16)

    row = lax.broadcasted_iota(jnp.int32, (BQ, BQ), 0)
    colm = lax.broadcasted_iota(jnp.int32, (BQ, BQ), 1)
    cmask = colm <= row
    acc[...] = jnp.zeros(acc.shape, F32)

    def head(h, par):
        PB = 512
        for r in range(0, S, PB):
            kv = _nn(c[r:r + PB, :], wpair[h])
            ks[r:r + PB, :] = kv[:, :D].astype(BF16)
            vs[r:r + PB, :] = kv[:, D:].astype(BF16)
        woh = wo[h]
        for i in range(NQ):
            L = (i + 1) * BQ
            q = qs[h, i * BQ:(i + 1) * BQ, :]
            HB = BQ // 2
            s_t = jnp.concatenate([_nt(q[:HB], ks[L - BQ:L - HB, :]),
                                   jnp.zeros((HB, HB), F32)], axis=1)
            s_d = jnp.where(cmask, jnp.concatenate([s_t, _nt(q[HB:], ks[L - BQ:L, :])], axis=0), -1e9)
            mx = jnp.max(s_d, axis=1, keepdims=True)
            if i > 0:
                s_o = _nt(q, ks[0:L - BQ, :])
                mx = jnp.maximum(mx, jnp.max(s_o, axis=1, keepdims=True))
            p_d = jnp.exp(s_d - mx)
            l = jnp.sum(p_d, axis=1, keepdims=True)
            p_d = p_d.astype(BF16)
            ctx = jnp.concatenate([_nn(p_d[:HB, :HB], vs[L - BQ:L - HB, :]),
                                   _nn(p_d[HB:], vs[L - BQ:L, :])], axis=0)
            if i > 0:
                p_o = jnp.exp(s_o - mx)
                l = l + jnp.sum(p_o, axis=1, keepdims=True)
                ctx = ctx + _nn(p_o.astype(BF16), vs[0:L - BQ, :])
            ctx = (ctx * (1.0 / l)).astype(BF16)
            acc[i * BQ:(i + 1) * BQ, :] += _nt(ctx, woh)

    sh = shift_ref[...].astype(F32)
    shb = [jnp.broadcast_to(sh[:, s_:s_ + 1], (DA, T)) for s_ in range(4)]
    lane = lax.broadcasted_iota(jnp.int32, (DA, T), 1)
    dd = jnp.broadcast_to(ssmd_ref[...].astype(F32), (DA, T))
    R = 64
    state = {"rprev": None}

    def a_fwd(j):
        kc = ak[:, j * T:(j + 1) * T].astype(F32)
        rcur = [pltpu.roll(kc, s_, 1) for s_ in range(1, 4)]
        acc_k = kc * shb[0]
        for s_ in range(1, 4):
            fill = 0.0 if state["rprev"] is None else state["rprev"][s_ - 1]
            acc_k = acc_k + jnp.where(lane >= s_, rcur[s_ - 1], fill) * shb[s_]
        state["rprev"] = rcur
        kvb = (acc_k * av[:, j * T:(j + 1) * T].astype(F32)).astype(BF16)
        kvs[:, j * T:(j + 1) * T] = kvb
        xs[j] = _nn(kvb, fwd)

    def a_prod(i, r):
        zr = jnp.zeros((R, T), F32)
        zi = jnp.zeros((R, T), F32)
        for j in range(i + 1):
            xr = xs[j, r:r + R, :T]
            xi = xs[j, r:r + R, T:]
            gr = gs[i - j, r:r + R, :T]
            gi = gs[i - j, r:r + R, T:]
            zr = zr + (xr * gr - xi * gi)
            zi = zi + (xr * gi + xi * gr)
        return jnp.concatenate([zr.astype(BF16), zi.astype(BF16)], axis=1)

    def a_inv(i, zs):
        y = _nn(jnp.concatenate(zs, axis=0), inv)
        y = y + kvs[:, i * T:(i + 1) * T].astype(F32) * dd
        o = aq[:, i * T:(i + 1) * T].astype(F32) * y
        obuf[i * T:(i + 1) * T, 0:DA] = o.T.astype(BF16)

    unpack_pair(wq32, M, 0, wqpair, 0)
    for h in range(H):
        if h == 2:
            for d in a_copies[1:]:
                d.wait()
        if h == 8:
            for d in b_copies:
                d.wait()
        chunks = [] if h < 2 else [h - 2] if h < 14 else [2 * h - 16, 2 * h - 15]
        if h % 2 == 0 and h + 2 < H:
            unpack_pair(wq32, M, h // 2 + 1, wqpair, 0, (h + 2) % 4)
        for c_ in chunks:
            a_fwd(c_)
        zs = {c_: [] for c_ in chunks}
        for n_, r in enumerate(range(0, S, 256)):
            qs[h, r:r + 256, :] = (_nn(x[r:r + 256, :], wqpair[h % 4]) * (D ** -0.5)).astype(BF16)
            if n_ * R < DA:
                for c_ in chunks:
                    zs[c_].append(a_prod(c_, n_ * R))
            if h >= 8:
                unpack_pair(wk32, n_ * 128 + 128, h - 8, wpair, 0, 2 * (h - 8), n_ * 128)
                unpack_pair(wv32, n_ * 128 + 128, h - 8, wpair, D, 2 * (h - 8), n_ * 128)
        for c_ in chunks:
            a_inv(c_, zs[c_])

    out_a = cp(obuf.at[:, 0:384], out_h.at[:, 0:384], sems.at[10])
    out_a.start()

    def hh(h, cc):
        head(h, 0)
        return cc
    lax.fori_loop(0, H, hh, 0)

    obuf[:, DA:] = acc[...].astype(BF16)
    out_b = cp(obuf.at[:, 384:], out_h.at[:, 384:], sems.at[11])
    out_b.start()
    out_a.wait()
    out_b.wait()


@jax.jit
def pallas_concat_heads__ssm_conv_h3__compressed_kv_cla__prompt_kernel(
    A_q, A_k, A_v, A_shift_k, A_ssm_k, A_ssm_D, B_x, B_c_kv, B_w_q, B_w_uk, B_w_uv, B_w_o,
):
    fwd, inv = _dft_consts()
    any_spec = pl.BlockSpec(memory_space=pl.ANY)
    vm = pl.BlockSpec(memory_space=pltpu.VMEM)
    out = pl.pallas_call(
        _kernel,
        out_shape=jax.ShapeDtypeStruct((S, DA + M), BF16),
        in_specs=[any_spec, any_spec, any_spec, vm, any_spec, vm,
                  any_spec, any_spec, any_spec, any_spec, any_spec, any_spec, vm, vm],
        out_specs=any_spec,
        scratch_shapes=[
            pltpu.VMEM((DA, S), BF16), pltpu.VMEM((DA, S), BF16), pltpu.VMEM((DA, S), BF16),
            pltpu.VMEM((DA, S), BF16),
            pltpu.VMEM((DA, S), BF16),
            pltpu.VMEM((NCH, DA, 2 * T), F32), pltpu.VMEM((NCH, DA, 2 * T), F32),
            pltpu.VMEM((S, DA + M), BF16),
            pltpu.VMEM((M, S), BF16), pltpu.VMEM((S, M), BF16), pltpu.VMEM((S, DC), BF16),
            pltpu.VMEM((2, M * H, 128), BF16), pltpu.VMEM((2, DC * H, 128), BF16),
            pltpu.VMEM((2, DC * H, 128), BF16),
            pltpu.VMEM((H, M, D), BF16),
            pltpu.VMEM((H, DC, 2 * D), BF16), pltpu.VMEM((4, M, D), BF16),
            pltpu.VMEM((H, S, D), BF16), pltpu.VMEM((S, D), BF16), pltpu.VMEM((S, D), BF16),
            pltpu.VMEM((S, M), F32),
            pltpu.SemaphoreType.DMA((18,)),
        ],
        compiler_params=pltpu.CompilerParams(vmem_limit_bytes=110 * 1024 * 1024),
    )(
        A_q.reshape(S, DA).T, A_k.reshape(S, DA).T, A_v.reshape(S, DA).T, A_shift_k, A_ssm_k,
        A_ssm_D.reshape(DA, 1), B_x.reshape(S, M).T, B_c_kv.reshape(S, DC),
        B_w_q.reshape(M * H, D), B_w_uk.reshape(DC * H, D), B_w_uv.reshape(DC * H, D), B_w_o.transpose(0, 2, 1),
        fwd, inv,
    )
    return out.reshape(1, S, DA + M)
```

```python
import functools
import numpy as np
import jax
import jax.numpy as jnp
from jax import lax
import jax.experimental.pallas as pl
import jax.experimental.pallas.tpu as pltpu

S = 2048
DA = 448
M = 448
H = 16
D = 256
DC = 1024
T = 128
NCH = S // T
BQ = 256
NQ = S // BQ

F32 = jnp.float32
BF16 = jnp.bfloat16


def _dft_consts():
    n = np.arange(T)
    k = np.arange(T)
    w = np.pi * (2 * k[:, None] + 1) * n[None, :] / (2 * T)
    fwd = np.concatenate([np.cos(w), -np.sin(w)], axis=0)
    inv = np.concatenate([np.cos(w).T, -np.sin(w).T], axis=1) / T
    return np.ascontiguousarray(fwd.T).astype(np.float32), np.ascontiguousarray(inv.T).astype(np.float32)


def _nt(a, b):
    return lax.dot_general(a, b, (((1,), (1,)), ((), ())), preferred_element_type=F32)


def _nn(a, b):
    return jnp.dot(a, b, preferred_element_type=F32)


def _kernel(aq_h, ak_h, av_h, shift_ref, ssmk_h, ssmd_ref, x_h, c_h, wq_h, wk_h, wv_h, wo_h,
            fwd_ref, inv_ref, out_h,
            aq, ak, av, hk, kvs, xs, gs, obuf,
            xt, x, c, wq, wk, wv, wo, wpair, wqpair, qs, ks, vs, acc, sems):
    cp = pltpu.make_async_copy
    a_copies = [cp(ssmk_h, hk, sems.at[0]), cp(ak_h, ak, sems.at[1]), cp(av_h, av, sems.at[2]),
                cp(aq_h, aq, sems.at[3])]
    b_copies = [cp(x_h, xt, sems.at[4]), cp(c_h, c, sems.at[5]), cp(wo_h, wo, sems.at[6])]
    for n_, (src, dst) in enumerate([(wq_h, wq), (wk_h, wk), (wv_h, wv)]):
        for half in range(2):
            b_copies.append(cp(src.at[:, half * 128:(half + 1) * 128], dst.at[half],
                               sems.at[12 + 2 * n_ + half]))
    q_copies = [b_copies[0]] + b_copies[3:5]
    b_copies = b_copies[1:3] + b_copies[5:]
    a_copies[0].start()
    for d in q_copies:
        d.start()

    fwd = fwd_ref[...].astype(BF16)
    inv = inv_ref[...].astype(BF16)
    sgn = jnp.where((lax.broadcasted_iota(jnp.int32, (DA, T), 1) & 1) == 0, 1.0, -1.0).astype(F32)

    a_copies[0].wait()
    prev = None
    for m_ in range(NCH):
        hf = _nn(hk[:, m_ * T:(m_ + 1) * T], fwd)
        if prev is None:
            gs[m_] = hf
        else:
            gs[m_, :, :T] = hf[:, :T] - sgn * prev[:, T:]
            gs[m_, :, T:] = hf[:, T:] + sgn * prev[:, :T]
        prev = hf

    for d in q_copies:
        d.wait()
    for d in a_copies[1:] + b_copies[2:4]:
        d.start()
    for r in range(0, S, 256):
        x[r:r + 256, :] = xt[:, r:r + 256].astype(F32).T.astype(BF16)
    wq32 = wq.bitcast(jnp.uint32)
    wk32 = wk.bitcast(jnp.uint32)
    wv32 = wv.bitcast(jnp.uint32)

    def unpack_pair(src32, n, j, dst, col, d0=0, r0=0):
        CH = 64
        for r in range(r0, n, CH):
          for half in range(2):
            w = src32[half, pl.ds(r * 8 + j, CH, stride=8), :]
            lo = pltpu.bitcast(w << 16, F32)
            hi = pltpu.bitcast(w & jnp.uint32(0xFFFF0000), F32)
            c0 = col + half * 128
            dst[d0, r:r + CH, c0:c0 + 128] = lo.astype(BF16)
            dst[d0 + 1, r:r + CH, c0:c0 + 128] = hi.astype(BF16)

    row = lax.broadcasted_iota(jnp.int32, (BQ, BQ), 0)
    colm = lax.broadcasted_iota(jnp.int32, (BQ, BQ), 1)
    cmask = colm <= row
    acc[...] = jnp.zeros(acc.shape, F32)

    def head(h, par):
        PB = 512
        for r in range(0, S, PB):
            kv = _nn(c[r:r + PB, :], wpair[h])
            ks[r:r + PB, :] = kv[:, :D].astype(BF16)
            vs[r:r + PB, :] = kv[:, D:].astype(BF16)
        woh = wo[h]
        for i in range(NQ):
            L = (i + 1) * BQ
            q = qs[h, i * BQ:(i + 1) * BQ, :]
            HB = BQ // 2
            s_t = jnp.concatenate([_nt(q[:HB], ks[L - BQ:L - HB, :]),
                                   jnp.zeros((HB, HB), F32)], axis=1)
            s_d = jnp.where(cmask, jnp.concatenate([s_t, _nt(q[HB:], ks[L - BQ:L, :])], axis=0), -1e9)
            mx = jnp.max(s_d, axis=1, keepdims=True)
            if i > 0:
                s_o = _nt(q, ks[0:L - BQ, :])
                mx = jnp.maximum(mx, jnp.max(s_o, axis=1, keepdims=True))
            p_d = jnp.exp(s_d - mx)
            l = jnp.sum(p_d, axis=1, keepdims=True)
            p_d = p_d.astype(BF16)
            ctx = jnp.concatenate([_nn(p_d[:HB, :HB], vs[L - BQ:L - HB, :]),
                                   _nn(p_d[HB:], vs[L - BQ:L, :])], axis=0)
            if i > 0:
                p_o = jnp.exp(s_o - mx)
                l = l + jnp.sum(p_o, axis=1, keepdims=True)
                ctx = ctx + _nn(p_o.astype(BF16), vs[0:L - BQ, :])
            ctx = (ctx * (1.0 / l)).astype(BF16)
            acc[i * BQ:(i + 1) * BQ, :] += _nt(ctx, woh)

    sh = shift_ref[...].astype(F32)
    shb = [jnp.broadcast_to(sh[:, s_:s_ + 1], (DA, T)) for s_ in range(4)]
    lane = lax.broadcasted_iota(jnp.int32, (DA, T), 1)
    dd = jnp.broadcast_to(ssmd_ref[...].astype(F32), (DA, T))
    R = 64
    state = {"rprev": None}

    def a_fwd(j):
        kc = ak[:, j * T:(j + 1) * T].astype(F32)
        rcur = [pltpu.roll(kc, s_, 1) for s_ in range(1, 4)]
        acc_k = kc * shb[0]
        for s_ in range(1, 4):
            fill = 0.0 if state["rprev"] is None else state["rprev"][s_ - 1]
            acc_k = acc_k + jnp.where(lane >= s_, rcur[s_ - 1], fill) * shb[s_]
        state["rprev"] = rcur
        kvb = (acc_k * av[:, j * T:(j + 1) * T].astype(F32)).astype(BF16)
        kvs[:, j * T:(j + 1) * T] = kvb
        xs[j] = _nn(kvb, fwd)

    def a_prod(i, r):
        zr = jnp.zeros((R, T), F32)
        zi = jnp.zeros((R, T), F32)
        for j in range(i + 1):
            xr = xs[j, r:r + R, :T]
            xi = xs[j, r:r + R, T:]
            gr = gs[i - j, r:r + R, :T]
            gi = gs[i - j, r:r + R, T:]
            zr = zr + (xr * gr - xi * gi)
            zi = zi + (xr * gi + xi * gr)
        return jnp.concatenate([zr.astype(BF16), zi.astype(BF16)], axis=1)

    def a_inv(i, zs):
        y = _nn(jnp.concatenate(zs, axis=0), inv)
        y = y + kvs[:, i * T:(i + 1) * T].astype(F32) * dd
        o = aq[:, i * T:(i + 1) * T].astype(F32) * y
        obuf[i * T:(i + 1) * T, 0:DA] = o.T.astype(BF16)

    unpack_pair(wq32, M, 0, wqpair, 0)
    for h in range(H):
        if h == 2:
            for d in a_copies[1:]:
                d.wait()
            for d in b_copies[4:]:
                d.start()
        if h == 8:
            for d in b_copies[2:]:
                d.wait()
            for d in b_copies[:2]:
                d.start()
        chunks = [] if h < 2 else [h - 2] if h < 14 else [2 * h - 16, 2 * h - 15]
        if h % 2 == 0 and h + 2 < H:
            unpack_pair(wq32, M, h // 2 + 1, wqpair, 0, (h + 2) % 4)
        for c_ in chunks:
            a_fwd(c_)
        zs = {c_: [] for c_ in chunks}
        for n_, r in enumerate(range(0, S, 256)):
            qs[h, r:r + 256, :] = (_nn(x[r:r + 256, :], wqpair[h % 4]) * (D ** -0.5)).astype(BF16)
            if n_ * R < DA:
                for c_ in chunks:
                    zs[c_].append(a_prod(c_, n_ * R))
            if h >= 8:
                unpack_pair(wk32, n_ * 128 + 128, h - 8, wpair, 0, 2 * (h - 8), n_ * 128)
                unpack_pair(wv32, n_ * 128 + 128, h - 8, wpair, D, 2 * (h - 8), n_ * 128)
        for c_ in chunks:
            a_inv(c_, zs[c_])

    out_a = cp(obuf.at[:, 0:384], out_h.at[:, 0:384], sems.at[10])
    out_a.start()
    for d in b_copies[:2]:
        d.wait()

    def hh(h, cc):
        head(h, 0)
        return cc
    lax.fori_loop(0, H, hh, 0)

    obuf[:, DA:] = acc[...].astype(BF16)
    out_b = cp(obuf.at[:, 384:], out_h.at[:, 384:], sems.at[11])
    out_b.start()
    out_a.wait()
    out_b.wait()


@jax.jit
def pallas_concat_heads__ssm_conv_h3__compressed_kv_cla__prompt_kernel(
    A_q, A_k, A_v, A_shift_k, A_ssm_k, A_ssm_D, B_x, B_c_kv, B_w_q, B_w_uk, B_w_uv, B_w_o,
):
    fwd, inv = _dft_consts()
    any_spec = pl.BlockSpec(memory_space=pl.ANY)
    vm = pl.BlockSpec(memory_space=pltpu.VMEM)
    out = pl.pallas_call(
        _kernel,
        out_shape=jax.ShapeDtypeStruct((S, DA + M), BF16),
        in_specs=[any_spec, any_spec, any_spec, vm, any_spec, vm,
                  any_spec, any_spec, any_spec, any_spec, any_spec, any_spec, vm, vm],
        out_specs=any_spec,
        scratch_shapes=[
            pltpu.VMEM((DA, S), BF16), pltpu.VMEM((DA, S), BF16), pltpu.VMEM((DA, S), BF16),
            pltpu.VMEM((DA, S), BF16),
            pltpu.VMEM((DA, S), BF16),
            pltpu.VMEM((NCH, DA, 2 * T), F32), pltpu.VMEM((NCH, DA, 2 * T), F32),
            pltpu.VMEM((S, DA + M), BF16),
            pltpu.VMEM((M, S), BF16), pltpu.VMEM((S, M), BF16), pltpu.VMEM((S, DC), BF16),
            pltpu.VMEM((2, M * H, 128), BF16), pltpu.VMEM((2, DC * H, 128), BF16),
            pltpu.VMEM((2, DC * H, 128), BF16),
            pltpu.VMEM((H, M, D), BF16),
            pltpu.VMEM((H, DC, 2 * D), BF16), pltpu.VMEM((4, M, D), BF16),
            pltpu.VMEM((H, S, D), BF16), pltpu.VMEM((S, D), BF16), pltpu.VMEM((S, D), BF16),
            pltpu.VMEM((S, M), F32),
            pltpu.SemaphoreType.DMA((18,)),
        ],
        compiler_params=pltpu.CompilerParams(vmem_limit_bytes=110 * 1024 * 1024),
    )(
        A_q.reshape(S, DA).T, A_k.reshape(S, DA).T, A_v.reshape(S, DA).T, A_shift_k, A_ssm_k,
        A_ssm_D.reshape(DA, 1), B_x.reshape(S, M).T, B_c_kv.reshape(S, DC),
        B_w_q.reshape(M * H, D), B_w_uk.reshape(DC * H, D), B_w_uv.reshape(DC * H, D), B_w_o.transpose(0, 2, 1),
        fwd, inv,
    )
    return out.reshape(1, S, DA + M)
```
